```python
import jax
import jax.numpy as jnp

def _softmax(x, axis=-1):
    return jax.nn.softmax(x, axis=axis)
def _gelu(x):
    return jax.nn.gelu(x, approximate=True)
def _silu(x):
    return jax.nn.silu(x)
def _sigmoid(x):
    return jax.nn.sigmoid(x)
def _layernorm(x, axis=-1, eps=1e-5):
    m = jnp.mean(x, axis=axis, keepdims=True)
    v = jnp.var(x, axis=axis, keepdims=True)
    return (x - m) / jnp.sqrt(v + eps)
def _scatter_add(tgt, idx, src, axis=0):
    return tgt.at[idx].add(src)
def _segment_sum(src, seg, n):
    return jax.ops.segment_sum(src, seg, n)
class _Rng:
    def __init__(self, key):
        self._k = key
    def _next(self):
        self._k, sub = jax.random.split(self._k)
        return sub
    def normal(self, shape):
        return jax.random.normal(self._next(), shape, dtype=jnp.bfloat16)
    def randint(self, lo, hi, shape):
        return jax.random.randint(self._next(), shape, lo, hi, dtype=jnp.int32)
    def uniform(self, shape, lo=0.0, hi=1.0):
        return jax.random.uniform(self._next(), shape, jnp.bfloat16, lo, hi)
    def permutation(self, n):
        return jax.random.permutation(self._next(), n)


kernel_name = 'standalone__qk_norm__prompt'

def setup_inputs():
    _rng = _Rng(jax.random.key(int.from_bytes(__import__("os").urandom(4), "little")))
    _w = (lambda a: (lambda t: t.astype(jnp.bfloat16) if jnp.issubdtype(t.dtype, jnp.floating) else t)(jnp.asarray(a)))
    B, H, S, D = 2, 32, 2048, 1024
    Dh = D // H
    return {
        "q": _w((lambda *s: _rng.normal(s) * 0.05)(B, H, S, Dh)),
        "k": _w((lambda *s: _rng.normal(s) * 0.05)(B, H, S, Dh)),
        "v": _w((lambda *s: _rng.normal(s) * 0.05)(B, H, S, Dh)),
        "t": _w(jnp.abs((lambda *s: _rng.normal(s) * 0.05)(H)) + 1.0),
    }

def reference(q, k, v, t):
    eps = 1e-6
    qn = q / (jnp.sqrt((q * q).sum(axis=-1, keepdims=True)) + eps)
    kn = k / (jnp.sqrt((k * k).sum(axis=-1, keepdims=True)) + eps)
    logits = jnp.einsum('bhqd,bhkd->bhqk', qn, kn) * t[None, :, None, None]
    attn = _softmax(logits, axis=-1)
    return jnp.einsum('bhqk,bhkd->bhqd', attn, v)
```

```python
import jax
import jax.numpy as jnp
from jax import lax
from jax.experimental import pallas as pl
from jax.experimental.pallas import tpu as pltpu

_LOG2E = 1.4426950408889634
_EPS = 1e-6
_T_SAFE = 16.0

_BQ = 512
_BK = 256
_SKEW = 3
_LATE = 3
_NS = 4

_F32 = jnp.float32
_BF16 = jnp.bfloat16


def _colsum8(p):
    return jnp.sum(p.reshape(p.shape[0] // 8, 8, p.shape[1]), axis=0)


def _make_kernel(G, H, D, S):
    NC = S // _BK
    NQ = S // _BQ
    KA = D + 16
    QLAST = slice((NQ - 1) * _BQ, NQ * _BQ)

    def kernel(t_ref, q_hbm, k_hbm, v_hbm, o_hbm,
               qb, kb, vb, ob, qa_ref, ka_ref, acc_ref, l_ref,
               q_sem, k_sem, v_sem, o_sem):

        def slot(h):
            return h & (_NS - 1)

        def clamp(h):
            return jnp.minimum(h, G - 1)

        def cp_q(h):
            return pltpu.make_async_copy(q_hbm.at[clamp(h)], qb.at[slot(h)], q_sem.at[slot(h)])

        def cp_k(h):
            return pltpu.make_async_copy(k_hbm.at[clamp(h)], kb.at[slot(h)], k_sem.at[slot(h)])

        def cp_v(h):
            return pltpu.make_async_copy(v_hbm.at[clamp(h)], vb.at[slot(h)], v_sem.at[slot(h)])

        def cp_o(h):
            return pltpu.make_async_copy(ob.at[slot(h)], o_hbm.at[h], o_sem.at[slot(h)])

        def scale_of(h):
            hh = clamp(h)
            hh = hh & (H - 1) if H & (H - 1) == 0 else lax.rem(hh, H)
            return t_ref[hh].astype(_F32) * _LOG2E

        def prep_q(s, ts, j):
            cols = slice(j * _BQ, (j + 1) * _BQ)
            q = qb[s, :, cols].astype(_F32)
            inv = ts / (jnp.sqrt(jnp.sum(q * q, axis=0, keepdims=True)) + _EPS)
            qa_ref[0:D, cols] = (q * inv).astype(_BF16)
            row = lax.broadcasted_iota(jnp.int32, (KA - D, _BQ), 0)
            qa_ref[D:KA, cols] = jnp.where(row == 0, -jnp.abs(ts), 0.0).astype(_BF16)

        def prep_k(s, c):
            cols = slice(c * _BK, (c + 1) * _BK)
            k = kb[s, :, cols].astype(_F32)
            inv = 1.0 / (jnp.sqrt(jnp.sum(k * k, axis=0, keepdims=True)) + _EPS)
            row = lax.broadcasted_iota(jnp.int32, (128 - D, _BK), 0)
            ext = jnp.where(row == 0, 1.0, 0.0)
            ka_ref[cols, :] = jnp.concatenate([k * inv, ext], axis=0).T.astype(_BF16)

        def prep_early(s, ts):
            for j in range(NQ):
                prep_q(s, ts, j)
            for c in range(NC - _LATE):
                prep_k(s, c)

        def finish_prev(h):
            inv = 1.0 / jnp.sum(l_ref[...], axis=0, keepdims=True)
            ob[slot(h + _NS - 1), :, QLAST] = (acc_ref[...] * inv).astype(ob.dtype)

        def refill(h):
            cp_q(h + 3).start()
            cp_k(h + 3).start()
            cp_v(h + 2).start()

            @pl.when(h > 0)
            def _():
                cp_o(h - 1).start()

        def bounded_head(h, ts_next):
            s, sn = slot(h), slot(h + 1)
            for c in range(NC - _LATE, NC):
                prep_k(s, c)
            finish_prev(h)
            probs = {}
            state = {}
            n_items = NQ * NC
            for n in range(n_items + _SKEW):
                if n < n_items:
                    j, c = divmod(n, NC)
                    if c == 0:
                        state[j] = dict(qa=qa_ref[:, j * _BQ:(j + 1) * _BQ], l=None, acc=None)
                    st = state[j]
                    sc = jnp.dot(ka_ref[c * _BK:(c + 1) * _BK, 0:KA], st["qa"],
                                 preferred_element_type=_F32)
                    p = jnp.exp2(sc)
                    lp = _colsum8(p)
                    st["l"] = lp if c == 0 else st["l"] + lp
                    probs[n] = p.astype(_BF16)
                    if j == NQ - 1 and c < NC - _LATE:
                        prep_k(sn, c)
                    if c == NC - 1:
                        prep_q(sn, ts_next, j)
                m = n - _SKEW
                if m >= 0:
                    j, c = divmod(m, NC)
                    st = state[j]
                    o = jnp.dot(vb[s, :, c * _BK:(c + 1) * _BK], probs.pop(m),
                                preferred_element_type=_F32)
                    st["acc"] = o if c == 0 else st["acc"] + o
                    if c == NC - 1:
                        if j < NQ - 1:
                            inv = 1.0 / jnp.sum(st["l"], axis=0, keepdims=True)
                            ob[s, :, j * _BQ:(j + 1) * _BQ] = (st["acc"] * inv).astype(ob.dtype)
                        else:
                            acc_ref[...] = st["acc"]
                            l_ref[...] = st["l"]
            refill(h)

        def true_max_head(h, ts_next):
            s, sn = slot(h), slot(h + 1)
            for c in range(NC - _LATE, NC):
                prep_k(s, c)
            finish_prev(h)

            def tile(q0):
                qa = qa_ref[0:D, pl.ds(q0, 128)]

                def logits(c):
                    k0 = pl.multiple_of(c * _BK, _BK)
                    return k0, jnp.dot(ka_ref[pl.ds(k0, _BK), 0:D], qa, preferred_element_type=_F32)

                def max_step(c, m):
                    _, sc = logits(c)
                    return jnp.maximum(m, jnp.max(sc.reshape(_BK // 8, 8, 128), axis=0))

                m = lax.fori_loop(0, NC, max_step, jnp.full((8, 128), -jnp.inf, _F32))
                m = jnp.max(m, axis=0, keepdims=True)

                def acc_step(c, carry):
                    acc, l = carry
                    k0, sc = logits(c)
                    p = jnp.exp2(sc - m)
                    o = jnp.dot(vb[s, :, pl.ds(k0, _BK)], p.astype(_BF16), preferred_element_type=_F32)
                    return acc + o, l + _colsum8(p)

                acc, l = lax.fori_loop(
                    0, NC, acc_step, (jnp.zeros((D, 128), _F32), jnp.zeros((8, 128), _F32)))
                return acc * (1.0 / jnp.sum(l, axis=0, keepdims=True))

            n_direct = (NQ - 1) * _BQ // 128

            def direct(i, carry):
                q0 = pl.multiple_of(i * 128, 128)
                ob[s, :, pl.ds(q0, 128)] = tile(q0).astype(ob.dtype)
                return carry

            lax.fori_loop(0, n_direct, direct, 0)

            def deferred(i, carry):
                a0 = pl.multiple_of(i * 128, 128)
                acc_ref[:, pl.ds(a0, 128)] = tile(pl.multiple_of(n_direct * 128 + a0, 128))
                return carry

            lax.fori_loop(0, _BQ // 128, deferred, 0)
            l_ref[...] = jnp.full((8, _BQ), 0.125, _F32)
            prep_early(sn, ts_next)
            refill(h)

        for h0 in range(3):
            cp_q(h0).start()
            cp_k(h0).start()
            if h0 < 2:
                cp_v(h0).start()
        acc_ref[...] = jnp.zeros(acc_ref.shape, _F32)
        l_ref[...] = jnp.ones(l_ref.shape, _F32)
        ts0 = scale_of(0)
        cp_q(0).wait()
        cp_k(0).wait()
        prep_early(0, ts0)

        def head(h, carry):
            ts_cur, ts_next = carry
            cp_v(h).wait()
            cp_q(h + 1).wait()
            cp_k(h + 1).wait()

            @pl.when(h >= 3)
            def _():
                cp_o(h - 3).wait()

            safe = jnp.abs(ts_cur) <= _T_SAFE * _LOG2E

            @pl.when(safe)
            def _():
                bounded_head(h, ts_next)

            @pl.when(jnp.logical_not(safe))
            def _():
                true_max_head(h, ts_next)

            return ts_next, scale_of(h + 2)

        lax.fori_loop(0, G, head, (ts0, scale_of(1)))

        finish_prev(G)
        cp_o(G - 1).start()
        for h1 in range(max(0, G - 3), G):
            cp_o(h1).wait()
        for h1 in (G + 1, G + 2):
            cp_q(h1).wait()
            cp_k(h1).wait()
        for h1 in (G, G + 1):
            cp_v(h1).wait()

    return kernel, KA


@jax.jit
def pallas_standalone__qk_norm__prompt_kernel(
    q: jax.Array,
    k: jax.Array,
    v: jax.Array,
    t: jax.Array,
):
    B, H, S, D = q.shape
    G = B * H
    assert S % _BQ == 0 and S % _BK == 0 and S // _BK > _LATE and D % 16 == 0 and D < 112
    qt, kt, vt = (jnp.swapaxes(x, 2, 3).reshape(G, D, S) for x in (q, k, v))
    kernel, KA = _make_kernel(G, H, D, S)
    hbm = pl.BlockSpec(memory_space=pl.ANY)
    io_slots = pltpu.VMEM((_NS, D, S), q.dtype)
    sems = pltpu.SemaphoreType.DMA((_NS,))
    out_t = pl.pallas_call(
        kernel,
        in_specs=[pl.BlockSpec(memory_space=pltpu.SMEM), hbm, hbm, hbm],
        out_specs=hbm,
        out_shape=jax.ShapeDtypeStruct((G, D, S), q.dtype),
        scratch_shapes=[
            io_slots, io_slots, io_slots, io_slots,
            pltpu.VMEM((KA, S), _BF16),
            pltpu.VMEM((S, 128), _BF16),
            pltpu.VMEM((D, _BQ), _F32),
            pltpu.VMEM((8, _BQ), _F32),
            sems, sems, sems, sems,
        ],
        compiler_params=pltpu.CompilerParams(
            vmem_limit_bytes=64 * 1024 * 1024,
            disable_bounds_checks=True,
        ),
    )(t, qt, kt, vt)
    return jnp.swapaxes(out_t.reshape(B, H, D, S), 2, 3)
```

```python
import jax
import jax.numpy as jnp
from jax import lax
from jax.experimental import pallas as pl
from jax.experimental.pallas import tpu as pltpu

_LOG2E = 1.4426950408889634
_EPS = 1e-6
_T_SAFE = 16.0

_BQ = 512
_BK = 512
_SKEW = 2
_LATE = 2
_PRING = 4
_HPI = 2

_F32 = jnp.float32
_BF16 = jnp.bfloat16


def _pack(x):
    return pltpu.bitcast(x.astype(_BF16), jnp.uint32)


def _unpack(x):
    return pltpu.bitcast(x, _BF16)


def _colsum8(p):
    return jnp.sum(p.reshape(p.shape[0] // 8, 8, p.shape[1]), axis=0)


def _make_kernel(G, H, D, S, HPI):
    NG = G // HPI
    NC = S // _BK
    NQ = S // _BQ
    KA = D + 16
    QLAST = slice((NQ - 1) * _BQ, NQ * _BQ)
    NSLOT = 4 * HPI

    def kernel(t_hbm, q_hbm, k_hbm, v_hbm, o_hbm,
               qb, kb, vb, ob, qa_ref, ka_ref, p_ref, acc_ref, l_ref,
               q_sem, k_sem, v_sem, o_sem, t_ref, ts_ref, t_sem):

        def slot(h):
            return h & (NSLOT - 1)

        def cp_in(hbm, buf, sem, h, g):
            return pltpu.make_async_copy(hbm.at[jnp.minimum(h, G - 1)], buf.at[slot(h)],
                                         sem.at[g & 3])

        def in_copies(g):
            out = []
            for i in range(HPI):
                h = g * HPI + i
                out.append((h, cp_in(v_hbm, vb, v_sem, h, g)))
                out.append((h, cp_in(q_hbm, qb, q_sem, h + 1, g)))
                out.append((h, cp_in(k_hbm, kb, k_sem, h + 1, g)))
            return out

        def fetch_for(g):
            for h, cp in in_copies(g):
                if isinstance(h, int):
                    if h < G:
                        cp.start()
                else:
                    pl.when(h < G)(cp.start)

        def cp_o(h, g):
            return pltpu.make_async_copy(ob.at[slot(h)], o_hbm.at[h], o_sem.at[g & 3])

        def scale_of(h):
            return ts_ref[h & (H - 1) if H & (H - 1) == 0 else lax.rem(h, H)]

        def prep_q(s, ts, j):
            cols = slice(j * _BQ, (j + 1) * _BQ)
            q = qb[s, :, cols].astype(_F32)
            inv = ts / (jnp.sqrt(jnp.sum(q * q, axis=0, keepdims=True)) + _EPS)
            qa_ref[0:D // 2, cols] = _pack(q * inv)
            row = lax.broadcasted_iota(jnp.int32, (KA - D, _BQ), 0)
            qa_ref[D // 2:KA // 2, cols] = _pack(jnp.where(row == 0, -jnp.abs(ts), 0.0))

        def prep_k(s, c):
            cols = slice(c * _BK, (c + 1) * _BK)
            k = kb[s, :, cols].astype(_F32)
            inv = 1.0 / (jnp.sqrt(jnp.sum(k * k, axis=0, keepdims=True)) + _EPS)
            row = lax.broadcasted_iota(jnp.int32, (128 - D, _BK), 0)
            ext = jnp.where(row == 0, 1.0, 0.0)
            ka_ref[c * _BK // 2:(c + 1) * _BK // 2, :] = _pack(jnp.concatenate([k * inv, ext], axis=0).T)

        def prep_early(h):
            s, ts = slot(h), scale_of(h)
            for j in range(NQ):
                prep_q(s, ts, j)
            for c in range(NC - _LATE):
                prep_k(s, c)

        def finish(h):
            inv = 1.0 / jnp.sum(l_ref[...], axis=0, keepdims=True)
            ob[slot(h), :, QLAST] = (acc_ref[...] * inv).astype(ob.dtype)

        def finish_prev(g):
            finish(g * HPI - 1 + NSLOT)

        def write_back(g):
            pl.when(g > 0)(cp_o(g * HPI - 1, g).start)
            for i in range(HPI - 1):
                cp_o(g * HPI + i, g).start()

        def write_back_wait(g):
            if isinstance(g, int):
                if g > 0:
                    cp_o(g * HPI - 1, g).wait()
            else:
                pl.when(g > 0)(cp_o(g * HPI - 1, g).wait)
            for i in range(HPI - 1):
                cp_o(g * HPI + i, g).wait()

        def bounded_group(g, ts):
            slots = [slot(g * HPI + i) for i in range(HPI + 1)]
            finish_prev(g)
            state = {}
            per_head = NQ * NC
            n_items = HPI * per_head
            for n in range(n_items + _SKEW):
                if n < n_items:
                    i, r = divmod(n, per_head)
                    j, c = divmod(r, NC)
                    if r == 0:
                        for cl in range(NC - _LATE, NC):
                            prep_k(slots[i], cl)
                    if c == 0:
                        state[i, j] = dict(qa=_unpack(qa_ref[:, j * _BQ:(j + 1) * _BQ]), l=None, acc=None)
                    st = state[i, j]
                    sc = jnp.dot(_unpack(ka_ref[c * _BK // 2:(c + 1) * _BK // 2, :])[:, 0:KA], st["qa"],
                                 preferred_element_type=_F32)
                    p = jnp.exp2(sc)
                    lp = _colsum8(p)
                    st["l"] = lp if c == 0 else st["l"] + lp
                    p_ref[n % _PRING] = _pack(p)
                    if j == NQ - 1 and c < NC - _LATE:
                        prep_k(slots[i + 1], c)
                    if c == NC - 1:
                        prep_q(slots[i + 1], ts[i + 1], j)
                m = n - _SKEW
                if m >= 0:
                    i, r = divmod(m, per_head)
                    j, c = divmod(r, NC)
                    st = state[i, j]
                    o = jnp.dot(vb[slots[i], :, c * _BK:(c + 1) * _BK], _unpack(p_ref[m % _PRING]),
                                preferred_element_type=_F32)
                    st["acc"] = o if c == 0 else st["acc"] + o
                    if c == NC - 1:
                        if m < n_items - 1:
                            inv = 1.0 / jnp.sum(st["l"], axis=0, keepdims=True)
                            ob[slots[i], :, j * _BQ:(j + 1) * _BQ] = (st["acc"] * inv).astype(ob.dtype)
                        else:
                            acc_ref[...] = st["acc"]
                            l_ref[...] = st["l"]
            fetch_for(g + 2)
            write_back(g)

        def true_max_group(g):
            finish_prev(g)

            def head(h, carry):
                s, ts = slot(h), scale_of(h)
                for j in range(NQ):
                    prep_q(s, ts, j)
                for c in range(NC):
                    prep_k(s, c)

                def tile(jt, carry):
                    q0 = pl.multiple_of(jt * 128, 128)
                    qa = _unpack(qa_ref[0:D // 2, pl.ds(q0, 128)])

                    def logits(c):
                        k0 = pl.multiple_of(c * _BK, _BK)
                        kn = _unpack(ka_ref[pl.ds(pl.multiple_of(c * (_BK // 2), _BK // 2), _BK // 2), :])
                        return k0, jnp.dot(kn[:, 0:D], qa,
                                           preferred_element_type=_F32)

                    def max_step(c, m):
                        _, sc = logits(c)
                        return jnp.maximum(m, jnp.max(sc.reshape(_BK // 8, 8, 128), axis=0))

                    m = lax.fori_loop(0, NC, max_step, jnp.full((8, 128), -jnp.inf, _F32))
                    m = jnp.max(m, axis=0, keepdims=True)

                    def acc_step(c, acc_l):
                        acc, l = acc_l
                        k0, sc = logits(c)
                        p = jnp.exp2(sc - m)
                        o = jnp.dot(vb[s, :, pl.ds(k0, _BK)], p.astype(_BF16),
                                    preferred_element_type=_F32)
                        return acc + o, l + _colsum8(p)

                    acc, l = lax.fori_loop(
                        0, NC, acc_step, (jnp.zeros((D, 128), _F32), jnp.zeros((8, 128), _F32)))
                    inv = 1.0 / jnp.sum(l, axis=0, keepdims=True)
                    ob[s, :, pl.ds(q0, 128)] = (acc * inv).astype(ob.dtype)
                    return carry

                return lax.fori_loop(0, S // 128, tile, carry)

            lax.fori_loop(g * HPI, (g + 1) * HPI, head, 0)
            acc_ref[...] = ob[slot(g * HPI + HPI - 1), :, QLAST].astype(_F32)
            l_ref[...] = jnp.full((8, _BQ), 0.125, _F32)
            prep_early((g + 1) * HPI)
            fetch_for(g + 2)
            write_back(g)

        cp_t = pltpu.make_async_copy(t_hbm, t_ref, t_sem)
        cp_t.start()
        cp_q0 = cp_in(q_hbm, qb, q_sem, 0, 3)
        cp_k0 = cp_in(k_hbm, kb, k_sem, 0, 3)
        cp_q0.start()
        cp_k0.start()
        fetch_for(0)
        fetch_for(1)
        acc_ref[...] = jnp.zeros(acc_ref.shape, _F32)
        l_ref[...] = jnp.ones(l_ref.shape, _F32)
        cp_t.wait()
        for i in range(H):
            ts_ref[i] = t_ref[i].astype(_F32) * _LOG2E
        cp_q0.wait()
        cp_k0.wait()
        prep_early(0)

        def group(g, carry):
            ts = [scale_of(g * HPI + i) for i in range(HPI + 1)]
            for _, cp in in_copies(g):
                cp.wait()

            @pl.when(g >= 3)
            def _():
                write_back_wait(g - 3)

            safe = jnp.abs(ts[0]) <= _T_SAFE * _LOG2E
            for i in range(1, HPI):
                safe = jnp.logical_and(safe, jnp.abs(ts[i]) <= _T_SAFE * _LOG2E)
            lax.cond(jnp.logical_not(safe),
                     lambda: true_max_group(g),
                     lambda: bounded_group(g, ts))
            return carry

        lax.fori_loop(0, NG, group, 0)

        finish_prev(NG)
        cp_o(G - 1, NG).start()
        for g in range(max(0, NG - 3), NG):
            write_back_wait(g)
        cp_o(G - 1, NG).wait()

    return kernel, KA


@jax.jit
def pallas_standalone__qk_norm__prompt_kernel(
    q: jax.Array,
    k: jax.Array,
    v: jax.Array,
    t: jax.Array,
):
    B, H, S, D = q.shape
    G = B * H
    assert S % _BQ == 0 and S % _BK == 0 and S // _BK > _LATE and D % 16 == 0 and D < 112
    qt, kt, vt = (jnp.swapaxes(x, 2, 3).reshape(G, D, S) for x in (q, k, v))
    HPI = _HPI if G % _HPI == 0 else 1
    kernel, KA = _make_kernel(G, H, D, S, HPI)
    hbm = pl.BlockSpec(memory_space=pl.ANY)
    io_slots = pltpu.VMEM((4 * HPI, D, S), q.dtype)
    sems = pltpu.SemaphoreType.DMA((4,))
    out_t = pl.pallas_call(
        kernel,
        in_specs=[hbm, hbm, hbm, hbm],
        out_specs=hbm,
        out_shape=jax.ShapeDtypeStruct((G, D, S), q.dtype),
        scratch_shapes=[
            io_slots, io_slots, io_slots, io_slots,
            pltpu.VMEM((KA // 2, S), jnp.uint32),
            pltpu.VMEM((S // 2, 128), jnp.uint32),
            pltpu.VMEM((_PRING, _BK // 2, _BQ), jnp.uint32),
            pltpu.VMEM((D, _BQ), _F32),
            pltpu.VMEM((8, _BQ), _F32),
            sems, sems, sems, sems,
            pltpu.SMEM((H,), t.dtype),
            pltpu.SMEM((H,), _F32),
            pltpu.SemaphoreType.DMA(()),
        ],
        compiler_params=pltpu.CompilerParams(vmem_limit_bytes=64 * 1024 * 1024),
    )(t, qt, kt, vt)
    return jnp.swapaxes(out_t.reshape(B, H, D, S), 2, 3)
```

```python
import jax
import jax.numpy as jnp
from jax import lax
from jax.experimental import pallas as pl
from jax.experimental.pallas import tpu as pltpu

_LOG2E = 1.4426950408889634
_EPS = 1e-6
_T_SAFE = 16.0

_BQ = 512
_BK = 512
_SKEW = 2
_LATE = 2
_PRING = 4
_HPI = 2

_F32 = jnp.float32
_BF16 = jnp.bfloat16


def _pack(x):
    return pltpu.bitcast(x.astype(_BF16), jnp.uint32)


def _unpack(x):
    return pltpu.bitcast(x, _BF16)


def _colsum8(p):
    return jnp.sum(p.reshape(p.shape[0] // 8, 8, p.shape[1]), axis=0)


def _make_kernel(G, H, D, S, HPI):
    NG = G // HPI
    NC = S // _BK
    NQ = S // _BQ
    KA = D + 16
    QLAST = slice((NQ - 1) * _BQ, NQ * _BQ)
    NSLOT = 4 * HPI

    def kernel(t_hbm, q_hbm, k_hbm, v_hbm, o_hbm,
               qb, kb, vb, ob, qa_ref, ka_ref, p_ref, acc_ref, l_ref,
               q_sem, k_sem, v_sem, o_sem, t_ref, ts_ref, t_sem):

        def slot(h):
            return h & (NSLOT - 1)

        def cp_in(hbm, buf, sem, h, g):
            return pltpu.make_async_copy(hbm.at[jnp.minimum(h, G - 1)], buf.at[slot(h)],
                                         sem.at[g & 3])

        def in_copies(g):
            out = []
            for i in range(HPI):
                h = g * HPI + i
                out.append((h, cp_in(v_hbm, vb, v_sem, h, g)))
                out.append((h, cp_in(q_hbm, qb, q_sem, h + 1, g)))
                out.append((h, cp_in(k_hbm, kb, k_sem, h + 1, g)))
            return out

        def fetch_for(g):
            for h, cp in in_copies(g):
                if isinstance(h, int):
                    if h < G:
                        cp.start()
                else:
                    pl.when(h < G)(cp.start)

        def cp_o(h, g):
            return pltpu.make_async_copy(ob.at[slot(h)], o_hbm.at[h], o_sem.at[g & 3])

        def head_of(h):
            return h & (H - 1) if H & (H - 1) == 0 else lax.rem(h, H)

        def scale_of(h):
            return ts_ref[head_of(h)]

        def prep_q(s, ts, j):
            cols = slice(j * _BQ, (j + 1) * _BQ)
            q = qb[s, :, cols].astype(_F32)
            inv = ts / (jnp.sqrt(jnp.sum(q * q, axis=0, keepdims=True)) + _EPS)
            qa_ref[0:D // 2, cols] = _pack(q * inv)
            row = lax.broadcasted_iota(jnp.int32, (KA - D, _BQ), 0)
            qa_ref[D // 2:KA // 2, cols] = _pack(jnp.where(row == 0, -jnp.abs(ts), 0.0))

        def prep_k(s, c):
            cols = slice(c * _BK, (c + 1) * _BK)
            k = kb[s, :, cols].astype(_F32)
            inv = 1.0 / (jnp.sqrt(jnp.sum(k * k, axis=0, keepdims=True)) + _EPS)
            row = lax.broadcasted_iota(jnp.int32, (128 - D, _BK), 0)
            ext = jnp.where(row == 0, 1.0, 0.0)
            ka_ref[c * _BK // 2:(c + 1) * _BK // 2, :] = _pack(jnp.concatenate([k * inv, ext], axis=0).T)

        def prep_early(h):
            s, ts = slot(h), scale_of(h)
            for j in range(NQ):
                prep_q(s, ts, j)
            for c in range(NC - _LATE):
                prep_k(s, c)

        def finish(h):
            inv = 1.0 / jnp.sum(l_ref[...], axis=0, keepdims=True)
            ob[slot(h), :, QLAST] = (acc_ref[...] * inv).astype(ob.dtype)

        def finish_prev(g):
            finish(g * HPI - 1 + NSLOT)

        def write_back(g):
            pl.when(g > 0)(cp_o(g * HPI - 1, g).start)
            for i in range(HPI - 1):
                cp_o(g * HPI + i, g).start()

        def write_back_wait(g):
            if isinstance(g, int):
                if g > 0:
                    cp_o(g * HPI - 1, g).wait()
            else:
                pl.when(g > 0)(cp_o(g * HPI - 1, g).wait)
            for i in range(HPI - 1):
                cp_o(g * HPI + i, g).wait()

        def bounded_group(g, ts):
            slots = [slot(g * HPI + i) for i in range(HPI + 1)]
            finish_prev(g)
            state = {}
            per_head = NQ * NC
            n_items = HPI * per_head
            for n in range(n_items + _SKEW):
                if n < n_items:
                    i, r = divmod(n, per_head)
                    j, c = divmod(r, NC)
                    if r == 0:
                        for cl in range(NC - _LATE, NC):
                            prep_k(slots[i], cl)
                    if c == 0:
                        state[i, j] = dict(qa=_unpack(qa_ref[:, j * _BQ:(j + 1) * _BQ]), l=None, acc=None)
                    st = state[i, j]
                    sc = jnp.dot(_unpack(ka_ref[c * _BK // 2:(c + 1) * _BK // 2, :])[:, 0:KA], st["qa"],
                                 preferred_element_type=_F32)
                    p = jnp.exp2(sc)
                    lp = _colsum8(p)
                    st["l"] = lp if c == 0 else st["l"] + lp
                    p_ref[n % _PRING] = _pack(p)
                    if j == NQ - 1 and c < NC - _LATE:
                        prep_k(slots[i + 1], c)
                    if c == NC - 1:
                        prep_q(slots[i + 1], ts[i + 1], j)
                m = n - _SKEW
                if m >= 0:
                    i, r = divmod(m, per_head)
                    j, c = divmod(r, NC)
                    st = state[i, j]
                    o = jnp.dot(vb[slots[i], :, c * _BK:(c + 1) * _BK], _unpack(p_ref[m % _PRING]),
                                preferred_element_type=_F32)
                    st["acc"] = o if c == 0 else st["acc"] + o
                    if c == NC - 1:
                        if m < n_items - 1:
                            inv = 1.0 / jnp.sum(st["l"], axis=0, keepdims=True)
                            ob[slots[i], :, j * _BQ:(j + 1) * _BQ] = (st["acc"] * inv).astype(ob.dtype)
                        else:
                            acc_ref[...] = st["acc"]
                            l_ref[...] = st["l"]
            fetch_for(g + 2)
            write_back(g)

        def true_max_group(g):
            finish_prev(g)

            def head(h, carry):
                s = slot(h)
                temp = t_ref[head_of(h)].astype(_F32)
                for j in range(NQ):
                    prep_q(s, 1.0, j)
                for c in range(NC):
                    prep_k(s, c)

                def tile(jt, carry):
                    q0 = pl.multiple_of(jt * 128, 128)
                    qa = _unpack(qa_ref[0:D // 2, pl.ds(q0, 128)])

                    def logits(c):
                        k0 = pl.multiple_of(c * _BK, _BK)
                        kn = _unpack(ka_ref[pl.ds(pl.multiple_of(c * (_BK // 2), _BK // 2), _BK // 2), :])
                        return k0, jnp.dot(kn[:, 0:D], qa, preferred_element_type=_F32) * temp

                    def max_step(c, m):
                        _, sc = logits(c)
                        return jnp.maximum(m, jnp.max(sc.reshape(_BK // 8, 8, 128), axis=0))

                    m = lax.fori_loop(0, NC, max_step, jnp.full((8, 128), -jnp.inf, _F32))
                    m = jnp.max(m, axis=0, keepdims=True)

                    def acc_step(c, acc_l):
                        acc, l = acc_l
                        k0, sc = logits(c)
                        p = jnp.exp2((sc - m) * _LOG2E)
                        o = jnp.dot(vb[s, :, pl.ds(k0, _BK)], p.astype(_BF16),
                                    preferred_element_type=_F32)
                        return acc + o, l + _colsum8(p)

                    acc, l = lax.fori_loop(
                        0, NC, acc_step, (jnp.zeros((D, 128), _F32), jnp.zeros((8, 128), _F32)))
                    inv = 1.0 / jnp.sum(l, axis=0, keepdims=True)
                    ob[s, :, pl.ds(q0, 128)] = (acc * inv).astype(ob.dtype)
                    return carry

                return lax.fori_loop(0, S // 128, tile, carry)

            lax.fori_loop(g * HPI, (g + 1) * HPI, head, 0)
            acc_ref[...] = ob[slot(g * HPI + HPI - 1), :, QLAST].astype(_F32)
            l_ref[...] = jnp.full((8, _BQ), 0.125, _F32)
            prep_early((g + 1) * HPI)
            fetch_for(g + 2)
            write_back(g)

        cp_t = pltpu.make_async_copy(t_hbm, t_ref, t_sem)
        cp_t.start()
        cp_q0 = cp_in(q_hbm, qb, q_sem, 0, 3)
        cp_k0 = cp_in(k_hbm, kb, k_sem, 0, 3)
        cp_q0.start()
        cp_k0.start()
        fetch_for(0)
        fetch_for(1)
        acc_ref[...] = jnp.zeros(acc_ref.shape, _F32)
        l_ref[...] = jnp.ones(l_ref.shape, _F32)
        cp_t.wait()
        for i in range(H):
            ts_ref[i] = t_ref[i].astype(_F32) * _LOG2E
        cp_q0.wait()
        cp_k0.wait()
        prep_early(0)

        def group(g, carry):
            ts = [scale_of(g * HPI + i) for i in range(HPI + 1)]
            for _, cp in in_copies(g):
                cp.wait()

            @pl.when(g >= 3)
            def _():
                write_back_wait(g - 3)

            safe = jnp.abs(ts[0]) <= _T_SAFE * _LOG2E
            for i in range(1, HPI):
                safe = jnp.logical_and(safe, jnp.abs(ts[i]) <= _T_SAFE * _LOG2E)
            lax.cond(jnp.logical_not(safe),
                     lambda: true_max_group(g),
                     lambda: bounded_group(g, ts))
            return carry

        lax.fori_loop(0, NG, group, 0)

        finish_prev(NG)
        cp_o(G - 1, NG).start()
        for g in range(max(0, NG - 3), NG):
            write_back_wait(g)
        cp_o(G - 1, NG).wait()

    return kernel, KA


@jax.jit
def pallas_standalone__qk_norm__prompt_kernel(
    q: jax.Array,
    k: jax.Array,
    v: jax.Array,
    t: jax.Array,
):
    B, H, S, D = q.shape
    G = B * H
    assert S % _BQ == 0 and S % _BK == 0 and S // _BK > _LATE and D % 16 == 0 and D < 112
    qt, kt, vt = (jnp.swapaxes(x, 2, 3).reshape(G, D, S) for x in (q, k, v))
    HPI = _HPI if G % _HPI == 0 else 1
    kernel, KA = _make_kernel(G, H, D, S, HPI)
    hbm = pl.BlockSpec(memory_space=pl.ANY)
    io_slots = pltpu.VMEM((4 * HPI, D, S), q.dtype)
    sems = pltpu.SemaphoreType.DMA((4,))
    out_t = pl.pallas_call(
        kernel,
        in_specs=[hbm, hbm, hbm, hbm],
        out_specs=hbm,
        out_shape=jax.ShapeDtypeStruct((G, D, S), q.dtype),
        scratch_shapes=[
            io_slots, io_slots, io_slots, io_slots,
            pltpu.VMEM((KA // 2, S), jnp.uint32),
            pltpu.VMEM((S // 2, 128), jnp.uint32),
            pltpu.VMEM((_PRING, _BK // 2, _BQ), jnp.uint32),
            pltpu.VMEM((D, _BQ), _F32),
            pltpu.VMEM((8, _BQ), _F32),
            sems, sems, sems, sems,
            pltpu.SMEM((H,), t.dtype),
            pltpu.SMEM((H,), _F32),
            pltpu.SemaphoreType.DMA(()),
        ],
        compiler_params=pltpu.CompilerParams(vmem_limit_bytes=64 * 1024 * 1024),
    )(t, qt, kt, vt)
    return jnp.swapaxes(out_t.reshape(B, H, D, S), 2, 3)
```
